```python
import jax
import jax.numpy as jnp

def _softmax(x, axis=-1):
    return jax.nn.softmax(x, axis=axis)
def _gelu(x):
    return jax.nn.gelu(x, approximate=True)
def _silu(x):
    return jax.nn.silu(x)
def _sigmoid(x):
    return jax.nn.sigmoid(x)
def _layernorm(x, axis=-1, eps=1e-5):
    m = jnp.mean(x, axis=axis, keepdims=True)
    v = jnp.var(x, axis=axis, keepdims=True)
    return (x - m) / jnp.sqrt(v + eps)
def _scatter_add(tgt, idx, src, axis=0):
    return tgt.at[idx].add(src)
def _segment_sum(src, seg, n):
    return jax.ops.segment_sum(src, seg, n)
class _Rng:
    def __init__(self, key):
        self._k = key
    def _next(self):
        self._k, sub = jax.random.split(self._k)
        return sub
    def normal(self, shape):
        return jax.random.normal(self._next(), shape, dtype=jnp.bfloat16)
    def randint(self, lo, hi, shape):
        return jax.random.randint(self._next(), shape, lo, hi, dtype=jnp.int32)
    def uniform(self, shape, lo=0.0, hi=1.0):
        return jax.random.uniform(self._next(), shape, jnp.bfloat16, lo, hi)
    def permutation(self, n):
        return jax.random.permutation(self._next(), n)


kernel_name = 'parallel_sum__compressed_kv_cla__moe_arch_mod__prompt'

def _fwd_setup_inputs():
    _rng = _Rng(jax.random.key(int.from_bytes(__import__("os").urandom(4), "little")))
    _w = (lambda a: (lambda t: t.astype(jnp.bfloat16) if jnp.issubdtype(t.dtype, jnp.floating) else t)(jnp.asarray(a)))
    def _A_setup():
        B, H, Sq, Sk, D, M = 1, 32, 2048, 2048, 128, 576
        Dc = 4 * D
        return {
            "x": _w((lambda *s: _rng.normal(s) * 0.05)(B, Sq, M)),
            "c_kv": _w((lambda *s: _rng.normal(s) * 0.05)(B, Sk, Dc)),
            "w_q": _w((lambda *s: _rng.normal(s) * 0.05)(M, H, D) * (M ** -0.5)),
            "w_uk": _w((lambda *s: _rng.normal(s) * 0.05)(Dc, H, D) * (Dc ** -0.5)),
            "w_uv": _w((lambda *s: _rng.normal(s) * 0.05)(Dc, H, D) * (Dc ** -0.5)),
            "w_o": _w((lambda *s: _rng.normal(s) * 0.05)(H, D, M) * ((H * D) ** -0.5)),
        }
    _A_in = _A_setup()

    def _B_setup():
        B, S, D, F, C = 1, 2048, 576, 4608, 8
        return {
            "x": _w((lambda *s: _rng.normal(s) * 0.05)(B, S, D)),
            "w_r": _w((lambda *s: _rng.normal(s) * 0.05)(D)),
            "w_gate": _w((lambda *s: _rng.normal(s) * 0.05)(D, F)),
            "w_up": _w((lambda *s: _rng.normal(s) * 0.05)(D, F)),
            "w_down": _w((lambda *s: _rng.normal(s) * 0.05)(F, D)),
        }
    _B_in = _B_setup()

    return {
        "A_x": _A_in["x"],
        "A_c_kv": _A_in["c_kv"],
        "A_w_q": _A_in["w_q"],
        "A_w_uk": _A_in["w_uk"],
        "A_w_uv": _A_in["w_uv"],
        "A_w_o": _A_in["w_o"],
        "B_x": _B_in["x"],
        "B_w_r": _B_in["w_r"],
        "B_w_gate": _B_in["w_gate"],
        "B_w_up": _B_in["w_up"],
        "B_w_down": _B_in["w_down"],
    }

def _fwd_reference(A_x, A_c_kv, A_w_q, A_w_uk, A_w_uv, A_w_o, B_x, B_w_r, B_w_gate, B_w_up, B_w_down):
    def _A_ref(x, c_kv, w_q, w_uk, w_uv, w_o):
        B, Sq, M = x.shape[0], x.shape[1], x.shape[2]
        Sk = c_kv.shape[1]
        H, D = w_q.shape[1], w_q.shape[2]
        q = jnp.einsum("bqm,mhd->bhqd", x, w_q)
        k = jnp.einsum("bkc,chd->bhkd", c_kv, w_uk)
        v = jnp.einsum("bkc,chd->bhkd", c_kv, w_uv)
        scores = jnp.einsum("bhqd,bhkd->bhqk", q, k) * (D ** -0.5)
        off = Sk - Sq
        qi = jnp.arange(Sq)[:, None]
        kj = jnp.arange(Sk)[None, :]
        cmask = kj <= (qi + off)
        scores = jnp.where(cmask[None, None], scores, -1e9)
        p = _softmax(scores, axis=-1)
        ctx = jnp.einsum("bhqk,bhkd->bhqd", p, v)
        return jnp.einsum("bhqd,hdm->bqm", ctx, w_o)

    def _B_ref(x, w_r, w_gate, w_up, w_down):
        B, S, D = x.shape
        C = 8
        r = x @ w_r
        idx = jnp.argsort(jax.lax.stop_gradient(-r), axis=-1)[:, :C]
        idx_e = jnp.repeat(idx.reshape(B, C, 1), D, axis=2)
        x_sel = jnp.take_along_axis(x, idx_e, axis=1)
        g = _silu(x_sel @ w_gate)
        u = x_sel @ w_up
        y = (g * u) @ w_down
        r_sel = _sigmoid(jnp.take_along_axis(r, idx, axis=1))
        y = y * r_sel.reshape(B, C, 1)
        b_off = (jnp.arange(B) * S).reshape(B, 1)
        flat_idx = (idx + b_off).reshape(B * C)
        zero = (x * 0.0).reshape(B * S, D)
        upd = _scatter_add(zero, flat_idx, y.reshape(B * C, D), axis=0)
        return x + upd.reshape(B, S, D)

    x = A_x
    xn = _layernorm(x, axis=-1)
    return x + _A_ref(xn, A_c_kv, A_w_q, A_w_uk, A_w_uv, A_w_o) + _B_ref(xn, B_w_r, B_w_gate, B_w_up, B_w_down)


def setup_inputs():
    _inp = _fwd_setup_inputs()
    _gk = jax.random.fold_in(jax.random.key(int.from_bytes(__import__("os").urandom(4), "little")), 2**31 - 1)
    _shapes = [[1, 2048, 576]]
    _dtypes = ['bfloat16']
    _gks = jax.random.split(_gk, len(_shapes))
    _gs = [jax.random.normal(k, s, dtype=jnp.dtype(d)) * 0.05 for k, s, d in zip(_gks, _shapes, _dtypes)]
    _inp["grad_out"] = _gs[0]
    return _inp

def reference(A_x, A_c_kv, A_w_q, A_w_uk, A_w_uv, A_w_o, B_w_r, B_w_gate, B_w_up, B_w_down, B_x, grad_out):
    _const = dict(B_x=B_x)
    def _f(*_d):
        return _fwd_reference(**{'A_x': _d[0], 'A_c_kv': _d[1], 'A_w_q': _d[2], 'A_w_uk': _d[3], 'A_w_uv': _d[4], 'A_w_o': _d[5], 'B_w_r': _d[6], 'B_w_gate': _d[7], 'B_w_up': _d[8], 'B_w_down': _d[9], **_const})
    _out, _vjp = jax.vjp(_f, A_x, A_c_kv, A_w_q, A_w_uk, A_w_uv, A_w_o, B_w_r, B_w_gate, B_w_up, B_w_down)
    _grads = _vjp(grad_out)
    _out0 = jnp.asarray(_out)
    return (_out0, *[jnp.asarray(_g) for _g in _grads])
```

```python
import functools
import math
import os

import jax
import jax.numpy as jnp
from jax import lax
from jax.experimental import pallas as pl
from jax.experimental.pallas import tpu as pltpu

f32 = jnp.float32
bf16 = jnp.bfloat16
u32 = jnp.uint32
i32 = jnp.int32

S = 2048
M = 576
DC = 512
H = 32
D = 128
F = 4608
TOPC = 8
T = 128
NC = S // T
NP = NC // 2
NG = 4
NBLK = NG * (NG - 1) // 2
CP = 16
NX = F // T - H
FC = NX * T
MH, MQ = M // 2, M // 4
KH = DC // 2
KM, KR, KQ = 224, 448, 32
DH = D // 2
HS, GW = S // 2, S // 4

NN = (((1,), (0,)), ((), ()))
NT = (((1,), (1,)), ((), ()))

SCALE = D ** -0.5
LOG2E = math.log2(math.e)
LN2 = math.log(2.0)
EPS_B = 1.0013580322265625e-05

_env = lambda k, d: os.environ.get(k, d)
FAST = int(_env("FAST", 0))
DEBUG = int(_env("DEBUG", 0))
BC = int(_env("BC", 32))
DLY, DLY2 = int(_env("DLY", 4)), int(_env("DLY2", 3))
PSPL = [int(x) for x in _env("PSPL", "2,3,4,3").split(",")]
ORD = [_env("O%d" % i, d).split(",") for i, d in enumerate((
    "G0,G1,G2,s20,G3,q4,A,o1,A,o1,A,o1,A,o5,A,s21,s22,q4",
    "C1,V1,C0,s03,A,P,A,A,A,K1,s02,EH,V0,K0,E1,E0",
    "C1,A,V1,C0,A,A,A,P,EH,KH,V0,s01,E1,E0,K1,K0",
    "A,C1,V1,W,A,C0,A,P,EH,KH,V0,E1,E0,K1,K0",
    "C1,C0,V1,KH,P,V0,E1,E0,K1,K0"))]
LIGHT = _env("LIGHT", "chunk,first,second,job").split(",")
DLY3 = int(_env("DLY3", 4))
ALN = int(_env("ALN", 2))
CAP = dict(zip("GpAHTic", [int(x) for x in _env("CAP", "28,28,32,40,30,30,40").split(",")]))
COST = dict(chunk=BC // 2, first=34, second=44, group=36, flip=34)
PPOS, PGAP, PEND = int(_env("PPOS", 2)), int(_env("PGAP", 12)), int(_env("PEND", 0))
MD = [int(x) for x in _env("MD", "7,6,5,4").split(",")]
DPC = int(_env("DPC", 4))
KG, KD, Q0 = float(_env("KG", 0)), int(_env("KD", 2)), int(_env("Q0", 4))
TWO = int(_env("TWO", 0))
QPH = int(_env("QPH", 3))
GA = int(_env("GA", 1))
CA = int(_env("CA", -4))
ATK = int(_env("ATK", 1))
B2G = float(_env("B2G", 0))
B2S = int(_env("B2S", 0))
PAR1, PAR2 = int(_env("PAR1", 0)), int(_env("PAR2", 8))
G0, G1, G2, G3, G4, G5 = [float(x) for x in _env("GAPS", "1.5,1.6,1.5,1.85,7,7").split(",")]
WD = int(_env("WD", 306))
WD1 = int(_env("WD1", 360))
G6 = float(_env("G6", 1.6))
OD0, OD1 = int(_env("OD0", 183)), int(_env("OD1", 200))

COMB = (((1, 0), (1, 3)), ((1, 2), (1, 3)), ((1, 0),), ((1, 3),), ((1, 0), (1, 1)), ((1, 2), (-1, 0)),
        ((1, 1), (-1, 3)))
BORD = (0, 2, 6, 5, 3, 4, 1)
SUMI = {0: 0, 1: 1, 4: 2, 5: 3, 6: 4}


def _comb(i, blk):
    (_, b0), *rest = COMB[i]
    v = blk[b0]
    for sg, b in rest:
        v = v + blk[b] if sg > 0 else v - blk[b]
    return v


def _recombine(m):
    return (m[0] + m[3] - m[4] + m[6], m[2] + m[4], m[1] + m[3], m[0] - m[1] + m[2] + m[5])


LAM = (-0.375, 0.375, -1.5, 1.5)
PAIRS = [(i, k) for i in range(NG) for k in range(i + 1, NG)]
OFFD = [(i, k) for i in range(NG) for k in range(NG) if k != i]
PQ, PP, PR, PN = 0, NG, 2 * NG, 2 * NG + len(PAIRS)
NR = PN + len(OFFD)
HW = ([{(k, i): 1 if k == i else -1 for k in range(NG)} for i in range(NG)]
      + [{(i, k): 1 if k == i else -1 for k in range(NG)} for i in range(NG)]
      + [{(k, i): 1, (i, k): -1} for i, k in PAIRS] + [{ik: 1} for ik in OFFD])
HSC = [1.0] * PR + [1.0 / (LAM[k] - LAM[i]) for i, k in PAIRS + OFFD]
LSLOT = ([PP + i for i in range(NG)] + [PQ + i for i in range(NG)] + list(range(PR, PN))
         + [PN + OFFD.index((k, i)) for i, k in OFFD])
HSETS = (('d', PP, PN), ((0, 1), PN, PN + 6), ((2, 3), PN + 6, NR))


def _lin(coef, blk):
    groups = {}
    for key, c in coef.items():
        groups.setdefault(abs(c), []).append((c > 0, key))
    acc = None
    for mag, terms in sorted(groups.items(), key=lambda kv: kv[0] == 1.0):
        terms = sorted(terms, key=lambda tk: not tk[0])
        if mag == 1.0 and acc is not None:
            for sg, key in terms:
                acc = acc + blk(key) if sg else acc - blk(key)
            continue
        pos = terms[0][0]
        v = blk(terms[0][1])
        for sg, key in terms[1:]:
            v = v + blk(key) if sg == pos else v - blk(key)
        assert pos or mag != 1.0
        v = v if mag == 1.0 else v * (mag if pos else -mag)
        acc = v if acc is None else acc + v
    return acc


def _tile(c):
    return slice(T * c, T * (c + 1))


def _dtile(c, w=T):
    return pl.ds(pl.multiple_of(c * w, w), w)


def _tiles(x):
    return [x[:, _tile(k)] for k in range(x.shape[1] // T)]


def _cat(xs, axis=1):
    return xs[0] if len(xs) == 1 else jnp.concatenate(xs, axis=axis)


def _full(c):
    return jnp.full((8, T), c, f32)


def _gate(an, vs, rows):
    bad = an != an
    sel = {}
    for v in vs:
        if id(v) not in sel:
            sel[id(v)] = lax.select(bad, an, v)
    return _cat([_cat([sel[id(v)] for v in vs])] * (rows // 8), 0)


def _hk_job(u, v, left, kind, an):
    sg = 1.0 if left else -1.0
    if kind == 'r':
        return v * _gate(an, [_full(1.0)] * NG, 16)
    if kind == 'd':
        m = u + v * _gate(an, [_full(sg * l) for l in LAM], 16)
        d = _tiles(m)
        return _cat([m] + [d[i] + d[k] for i, k in PAIRS])
    lv = v * _gate(an, [_full(sg * LAM[kind[0]])] * NG, 16)
    out = []
    for i, m in zip(kind, (u + lv, u - lv)):
        m = _tiles(m)
        out += [m[i] + m[k] for k in range(NG) if k != i]
    return _cat(out)


def _hk_order(left):
    quads = [[(PQ if left else PP) + x] + [PN + OFFD.index((y, x) if left else (x, y)) for y in range(NG) if y != x]
             for x in range(NG)]
    return quads, list(range(PP, PR) if left else range(PQ, PP)), list(range(PR, PN))


def _hk_adjoint(n, left, put):
    own, other = (PQ, PP) if left else (PP, PQ)
    diag = []

    def first(an):
        p, r = _tiles(n(own, own + NG) * _gate(an, [_full(1.0)] * NG, 16)), _tiles(n(PR, PN))
        for x in range(NG):
            diag.append(functools.reduce(jnp.add, [p[x]] + [r[q] for q, ik in enumerate(PAIRS) if x in ik]))

    def second(x0, an):
        one = _gate(an, [_full(1.0)], 16)
        plain, mixed = [], []
        for x in (x0, x0 + 1):
            slot = lambda y: PN + OFFD.index((x, y) if left else (y, x))
            t = [diag[x] * one if y == x else n(slot(y), slot(y) + 1) for y in range(NG)]
            plain.append((t[0] + t[1]) + (t[2] + t[3]))
            lt = _lin(dict(enumerate(LAM)), lambda y: t[y])
            mixed.append(n(other + x, other + x + 1) + lt if left else n(other + x, other + x + 1) - lt)
        put(x0, *((mixed, plain) if left else (plain, mixed)))
    return [first, functools.partial(second, 0), functools.partial(second, 2)]


def _dot(a, b, dims=NN):
    return lax.dot_general(a, b, dims, preferred_element_type=f32)


def _rb(x):
    return x.astype(bf16).astype(f32)


def _fold(x):
    return x.reshape(x.shape[0] // 8, 8, x.shape[1])


def _colsum(x):
    return jnp.sum(jnp.sum(_fold(x), axis=0), axis=0, keepdims=True)


def _sigmoid_b(x):
    return _rb(1.0 / _rb(1.0 + _rb(jnp.exp(-x))))


def _half(word, hi):
    return pltpu.bitcast(word & jnp.uint32(0xFFFF0000) if hi else word << 16, f32)


def _word(lo, hi):
    return (pltpu.bitcast(_rb(lo), u32) >> 16) | pltpu.bitcast(_rb(hi), u32)


def _chunks(n, step):
    return [(a, min(a + step, n)) for a in range(0, n, step)]


class _Jobs:
    def __init__(self):
        self.now, self.q, self.done, self.credit = 0, [], {}, 0

    def push(self, jobs, gap=0.0, delay=0, key=None, front=False):
        new = [(self.now + delay + int(gap * n), f, key if n == len(jobs) - 1 else None) for n, f in enumerate(jobs)]
        self.q = new + self.q if front else self.q + new

    def sort(self):
        self.q.sort(key=lambda e: e[0])

    def tick(self, anchor, only=None, cap=None):
        self.now += 1
        if cap is not None:
            self.credit = min(self.credit + cap, cap)
            if self.credit <= 0:
                return True
        for n, (t0, f, key) in enumerate(self.q):
            name = getattr(f, 'func', f).__name__
            if only is None or name in only:
                if self.now < t0:
                    break
                del self.q[n]
                f(anchor())
                self.done[key] = self.now
                self.credit -= COST.get(name, 44)
                return True
        return False

    def need(self, key):
        if DEBUG:
            print("need", key, "now", self.now, "done", self.done.get(key), "left", len(self.q))
        assert key in self.done, key


def _kernel(xT_hbm, gT_hbm, c_hbm, wq_hbm, wuk_hbm, wuv_hbm, woT_hbm, wr_hbm, wg_hbm, wu_hbm, wd_hbm,
            outT_hbm, dxT_hbm, dc_hbm, dwq_hbm, dwuk_hbm, dwuv_hbm, dwoT_hbm, dwr_hbm, dwg_hbm, dwu_hbm, dwd_hbm,
            XS_, DX_, CS_, ZR_, CT_, ZC_, ZD_, rstd, AM, AC, TMP, NW,
            RAW, WA, WTc_, WTt_, WTf, WKc_, WC_,
            KV_, KVT_, QO_, DO2_, Sc0, Sc1, Sc2, Sc3, P_, DH_, PC_, DS_, DD_, HC_, XF, YF, Xc_, Yc_,
            stA, stB, stO, wf_in_, wt_in, wt_out,
            XB, ACT, keys, taken, onehot, selacc, xsel, dysel, updT, dxsT, srt, yacc, dxacc, wr_ref, dwr_ref, kidx,
            sem_in, sem_w, sem_dw, sem_fi, sem_ti, sem_to, sem_out):
    pb = lambda r, k: r.at[k].bitcast(bf16)
    wq_u, wuk_u, wuv_u, woT_u = [r.bitcast(u32) for r in (wq_hbm, wuk_hbm, wuv_hbm, woT_hbm)]
    dwq_u, dwuk_u, dwuv_u = [r.bitcast(u32) for r in (dwq_hbm, dwuk_hbm, dwuv_hbm)]
    copy = pltpu.make_async_copy

    RQ, RK, RO = 0, M, M + 2 * DC

    def w_start(j):
        sl = j & 1
        for src, r0, n in ((wq_u.at[:, j, :], RQ, M), (wuk_u.at[:, j, :], RK, DC), (wuv_u.at[:, j, :], RK + DC, DC),
                           (woT_u.at[2 * j], RO, MH), (woT_u.at[2 * j + 1], RO + MH, MH)):
            copy(src, RAW.at[sl, pl.ds(r0, n), :], sem_w.at[sl]).start()

    def w_wait(j):
        copy(RAW.at[j & 1], RAW.at[j & 1], sem_w.at[j & 1]).wait()

    def grad_copies(j, fam):
        if fam == 0:
            return [copy(stA.at[0], dwq_u.at[:, j, :], sem_dw.at[0]), copy(stB.at[0], dwuk_u.at[:, j, :], sem_dw.at[1])]
        return [copy(stO.at[1], dwoT_hbm.at[pl.ds(2 * j, 2)], sem_dw.at[2]),
                copy(stB.at[1], dwuv_u.at[:, j, :], sem_dw.at[3])]

    def fi_copies():
        return [copy(src.at[:, pl.ds(H * T, FC)], pb(wf_in_, i), sem_fi.at[0])
                for i, src in enumerate((wg_hbm, wu_hbm, wd_hbm))]

    def ti_start(hh):
        for i, src in enumerate((wg_hbm, wu_hbm, wd_hbm)):
            copy(src.bitcast(u32).at[:, _dtile(hh)], wt_in.at[hh & 1, i], sem_ti.at[hh & 1]).start()

    def ti_wait(sl):
        copy(wt_in.at[sl], wt_in.at[sl], sem_ti.at[sl]).wait()

    def to_start(sl, tile):
        for i, dst in enumerate((dwg_hbm, dwu_hbm, dwd_hbm)):
            copy(wt_out.at[sl, i], dst.bitcast(u32).at[:, _dtile(tile)], sem_to.at[sl]).start()

    def to_wait(sl):
        copy(wt_out.at[sl], wt_out.at[sl], sem_to.at[sl]).wait()

    def prep_jobs(hh, z):
        WTc, WTt = pb(WTc_, z), pb(WTt_, z)
        sl = lax.shift_right_logical(hh, 1) & 1

        def rows(k, r0, n, an):
            if k == 1:
                w = RAW[sl, pl.ds(pl.multiple_of(RO + (hh & 1) * MH + r0 // 2, 8), n // 2), :]
                w = w | pltpu.bitcast(_gate(an, [_full(0.0)], n // 2), u32)
                return pltpu.bitcast(w, bf16).astype(f32)
            base = (RQ, None, RK, RK + DC)[k] + r0
            sh = pltpu.bitcast(_gate(an, [_full(0.0)], 8), u32) + ((hh & 1) * 16).astype(u32)
            return pltpu.bitcast((RAW[sl, base:base + n, :] >> _cat([sh] * (n // 8), 0)) << 16, f32)

        def main(k, q, an):
            if k >= 2:
                wt = [rows(k, KH * q + T * u, T, an).T for u in range(2)]
                WTf[z, _tile(k - 2), KH * q:KH * (q + 1)] = _cat(wt)
                return wt[0][D - 8:D] + wt[1][D - 8:D]
            if q == 1:
                wt = [_cat([rows(k, KM * u + T, KM - T, an), rows(k, KR + KQ * u, KQ, an)], 0).T for u in range(2)]
            else:
                wt = [rows(k, KM * u, T, an).T for u in range(2)]
            blk = [wt[b // 2][DH * (b % 2):DH * (b % 2 + 1)] for b in range(4)]
            ops = [_comb(BORD[i], blk) for i in range(7)]
            if q == 1:
                wr, w2 = rows(k, KR, T, an).T, rows(k, KR - KQ, T, an).T
                lane = lax.broadcasted_iota(i32, (DH, T), 1)
                ext = (blk[0], 0.0, 0.0, blk[2], -w2[0:DH], -blk[0], wr[0:DH])
                ops = [jnp.where(lane < KM - T, o, e) for o, e in zip(ops, ext)]
                mix = wr[DH:D] + jnp.where(jnp.logical_and(lane >= 2 * KQ, lane < 3 * KQ), wr[0:DH], 0.0)
                WTt[:, _tile(k)] = _cat([wr, mix], 0).astype(bf16)
                wt = [wt[0] + wt[1], wr + w2]
            WTc[7 * DH * k:7 * DH * (k + 1), _tile(q)] = _cat(ops, 0).astype(bf16)
            return wt[0][D - 8:D] + wt[1][D - 8:D]

        def kv(m, r0, kind, s0, s1, an):
            lo, hi = [WTf[z, D * m + DH * u + r0:D * m + DH * u + r0 + 16, :] for u in range(2)]
            ops = [o if s < PR else o * HSC[LSLOT.index(s)]
                   for s, o in zip(range(s0, s1), _tiles(_hk_job(hi, lo, True, kind, an)))]
            pb(WKc_, z)[DH * m + r0:DH * m + r0 + 16, T * s0:T * s1] = _cat(ops).astype(bf16)
        return ([functools.partial(main, k, q) for k in (2, 3, 0, 1) for q in range(2)],
                [functools.partial(kv, m, r0, *hs)
                 for m in range(2) for r0 in range(0, DH, 16) for hs in (('r', 0, NG),) + HSETS])

    XS, DX, CS = pb(XS_, 0), pb(DX_, 0), pb(CS_, 0)
    XN, GT, CT = pb(ZR_, 0), pb(ZR_, 1), pb(CT_, 0)
    tok = lambda p: _dtile(p, 2 * T)
    grp = lambda g: _dtile(g, GW)
    x_copy = lambda p: copy(xT_hbm.at[:, tok(p)], XS.at[:, tok(p)], sem_in.at[p])
    g_copy = lambda p: copy(gT_hbm.at[:, tok(p)], GT.at[:, tok(p)], sem_in.at[p])
    c_copy = lambda p: copy(c_hbm.at[tok(p), :], CS.at[tok(p), :], sem_in.at[p])

    for p in range(NP):
        x_copy(p).start()
    wr_copy = copy(wr_hbm, wr_ref, sem_out.at[3])
    wr_copy.start()
    for r in (ACT, srt, yacc, dxacc, selacc, onehot, taken):
        r[...] = jnp.zeros(r.shape, f32)

    def gated(b, an):
        zero = pltpu.bitcast(_gate(an, [_full(0.0)] * (b.shape[1] // T), b.shape[0] // 2), u32)
        return pltpu.bitcast(pltpu.bitcast(b, u32) | zero, bf16)

    def zc_sums(k, Z, p, an=None):
        src, dst, kh = Z.at[:, tok(p)], pb(ZC_, k).at[:, _dtile(p)], KM if k < 2 else KH
        for r0 in range(0, kh, 32):
            lo, hi = [src[kh * rh + r0:kh * rh + r0 + 32, :] for rh in range(2)]
            lo, hi = [_tiles((b if an is None else gated(b, an)).astype(f32)) for b in (lo, hi)]
            for i, sl in SUMI.items():
                dst[KH * sl + r0:KH * sl + r0 + 32, :] = _comb(i, (lo[0], hi[0], lo[1], hi[1])).astype(bf16)
        if k < 2:
            for sl, q in ((0, 0), (2, 2), (3, 0), (4, 3)):
                dst[KH * sl + KM:KH * (sl + 1), :] = src[KR + KQ * q:KR + KQ * (q + 1), 0:T]
            ev, od = _tiles(src[KR + KQ:KR + 2 * KQ, :].astype(f32))
            dst[KH + KM:2 * KH, :] = (od - ev).astype(bf16)

    def zd_sums(k, Z, hr, g, r0, n, anchors=None):
        cut = hr - 16 * n
        src = Z.at[pl.ds(pl.multiple_of(r0, 16), NG * hr - cut), grp(g)]
        dst = pb(ZD_, k).at[pl.ds(pl.multiple_of(r0, 16), PN * hr - cut), _dtile(g)]
        for s in range(0, 16 * n, 16):
            blk = [src[hr * i + s:hr * i + s + 16, :] for i in range(NG)]
            if anchors:
                blk = [gated(b, anchors[s // 16]) for b in blk]
            blk = [_tiles(b.astype(f32)) for b in blk]
            for r in range(PN):
                dst[hr * r + s:hr * r + s + 16, :] = _lin(HW[r], lambda iq: blk[iq[0]][iq[1]]).astype(bf16)

    def x_step(p, carry):
        x_copy(p).wait()
        g_copy(p).start()
        def strips(n):
            xs = pb(XS_, jnp.minimum(n * p, 0)).at[:, tok(p)]
            return ((r0, xs[r0:r0 + 32, :].astype(f32)) for r0 in range(0, M, 32))
        mu = _colsum(functools.reduce(jnp.add, (x for _, x in strips(1)))) * (1.0 / M)
        mu32 = jnp.broadcast_to(mu, (32, 2 * T))
        var = _colsum(functools.reduce(jnp.add, (jnp.square(x - mu32) for _, x in strips(2)))) * (1.0 / M)
        rs = jnp.broadcast_to(1.0 / _rb(jnp.sqrt(_rb(_rb(var) + EPS_B))), (32, 2 * T))
        mu32, xn = _rb(mu32), XN.at[:, tok(p)]
        for r0, x in strips(3):
            xn[r0:r0 + 32, :] = (_rb(x - mu32) * rs).astype(bf16)
        rstd[:, tok(p)] = rs[0:8]
        zc_sums(0, XN, p)
        return carry
    lax.fori_loop(0, NP, x_step, None)

    wr_copy.wait()
    wr = jnp.broadcast_to(wr_ref[...].astype(f32).reshape(1, M), (CP, M)).astype(bf16)
    keys[...] = _rb(_dot(wr, XN[...])[0:8])

    def g_step(p, carry):
        g_copy(p).wait()
        c_copy(p).start()
        rev = (S - 1 - lax.broadcasted_iota(i32, (8, S), 1)).astype(f32)
        free = taken[...] == 0.0
        part = functools.reduce(jnp.maximum, _tiles(jnp.where(free, keys[...], -jnp.inf)))
        top = jnp.max(part, axis=1, keepdims=True)
        zc_sums(1, GT, p, part if GA else None)
        cand = jnp.logical_and(free, jnp.logical_not(keys[...] < top))
        part = functools.reduce(jnp.maximum, _tiles(jnp.where(cand, rev, -1.0)))
        pos = jnp.max(part, axis=1, keepdims=True)
        zd_sums(0, XN, MQ, lax.shift_right_logical(p, 1), (p & 1) * 64, 5, [part] * 5 if GA else None)
        hit = rev == pos
        row = lax.broadcasted_iota(i32, (8, S), 0) == p
        taken[...] = jnp.where(hit, 1.0, taken[...])
        onehot[0:8, :] = jnp.where(jnp.logical_and(hit, row), 1.0, onehot[0:8, :])
        srt[0:8, :] = jnp.where(row[:, 0:T], _sigmoid_b(jnp.broadcast_to(top, (8, T))), srt[0:8, :])
        kidx[p] = S - 1 - pos[0, 0].astype(i32)
        return carry
    lax.fori_loop(0, TOPC, g_step, None)

    w_start(0)
    ti_start(0)

    def c_step(p, carry):
        c_copy(p).wait()
        CT[:, tok(p)] = CS[tok(p), :].T
        idx = kidx[p]
        tl = _dtile(lax.shift_right_logical(idx, 7))
        ef = (lax.broadcasted_iota(i32, (T, T), 0) == (idx & (T - 1))).astype(f32)
        e = ef.astype(bf16)
        for (a, b) in ((0, MH), (MH, M)):
            xb = _dot(XN[a:b, tl], e)
            XB[p, a:b, :] = xb
            XB[TOPC + p, a:b, :] = _rb(_dot(GT[a:b, tl], e) * srt[pl.ds(p, 1), :])
        zd_sums(1, GT, MQ, lax.shift_right_logical(p, 1), (p & 1) * 64, 5,
                [xb[CA * s:CA * s + 8] for s in range(5)] if CA >= 0 else [ef[0:8]] * (-CA) + [xb[0:8]] * (5 + CA))
        oh = jnp.where(lax.broadcasted_iota(i32, (CP, T), 0) == p, onehot[:, tl], 0.0).astype(bf16)
        selacc[0] += _dot(oh, XN[:, tl], NT)
        selacc[1] += _dot(oh, GT[:, tl], NT)
        return carry
    lax.fori_loop(0, NP, c_step, None)

    def zd_step(g, carry):
        zd_sums(2, CT, T, g, 0, T // 16)
        return carry
    lax.fori_loop(0, NG, zd_step, None)
    w_wait(0)
    w_start(1)
    for cp in fi_copies():
        cp.start()
    for job in sum(prep_jobs(jnp.int32(0), 0), []):
        job(_full(0.0))
    xsel[...] = selacc[0].astype(bf16)
    dysel[...] = (selacc[1] * srt[:, 0:1]).astype(bf16)

    def moe_act(a, u, dh):
        a, u, dh = _rb(a), _rb(u), _rb(dh)
        sg = _sigmoid_b(a)
        g = _rb(a * sg)
        dg = _rb(dh * u)
        da = _rb(dg * sg) + _rb(_rb(a * dg) * _rb(sg * _rb(1.0 - sg)))
        return da.astype(bf16), (dh * g).astype(bf16), (g * u).astype(bf16)

    def store_act(slot, acts):
        for i, act in enumerate(acts):
            act = act.astype(f32)
            for c in range(TOPC):
                ACT[slot, TOPC * i + c] = jnp.broadcast_to(act[c:c + 1], (8, T))

    def moe_chunk():
        wg, wu, wd = [pb(wf_in_, i)[...] for i in range(3)]
        da, du, hh = moe_act(_dot(xsel[...], wg), _dot(xsel[...], wu), _dot(dysel[...], wd))
        for k in range(NX):
            store_act(2 + k, [v[:, _tile(k)] for v in (da, du, hh)])
        yacc[...] += _dot(hh, wd, NT)
        dxacc[...] += _dot(da, wg, NT) + _dot(du, wu, NT)

    def head_block(j, t):
        h = 2 * j + t
        z = jnp.minimum(j, 0)
        WTc, WTt, KV, KVT, QO, DO2, P, DH4, PC, DS, DD, HC = [
            pb(r, z) for r in (WTc_, WTt_, KV_, KVT_, QO_, DO2_, P_, DH_, PC_, DS_, DD_, HC_)]
        Scs = [r.at[z] for r in (Sc0, Sc1, Sc2, Sc3)]
        dQ_o, O_o, dK_o, dV_o = XF.at[t], XF.at[2 + t], YF.at[t], YF.at[2 + t]
        OUT = (dQ_o, O_o, dK_o, dV_o)
        st = {}
        jobs, side = _Jobs(), _Jobs()

        ti_wait(t)

        @pl.when(jnp.logical_and(t == 1, j + 1 < H // 2))
        def _():
            w_wait(j + 1)

        @pl.when(h + 1 < H)
        def _():
            ti_start(h + 1)

        @pl.when(jnp.logical_and(t == 0, j > 0))
        def _():
            for cp in grad_copies(j - 1, 0) + grad_copies(j - 1, 1):
                cp.start()
            to_start(0, h - 2)
            to_start(1, h - 1)

        @pl.when(jnp.logical_and(t == 0, jnp.logical_and(j >= 2, j < 2 + NX // 2)))
        def _():
            to_start(2, H + h - 4)
            to_start(3, H + h - 3)

        moe1 = [(i, k) for i in range(3) for k in _chunks(M, T)]
        moe2 = list(moe1)

        def moe_small(n):
            w = lambda i, a, b: pltpu.bitcast(wt_in[t, i, a // 2:b // 2, :], bf16)
            for _ in range(n):
                if moe1:
                    i, (a, b) = moe1.pop(0)
                    v = _dot((xsel, xsel, dysel)[i][:, a:b], w(i, a, b))
                    st['f', i] = v if a == 0 else st['f', i] + v
                    if not moe1:
                        st['act'] = moe_act(st['f', 0], st['f', 1], st['f', 2])
                        store_act(t, st['act'])
                        return
                elif moe2:
                    i, (a, b) = moe2.pop(0)
                    acc = yacc if i == 2 else dxacc
                    acc[:, a:b] += _dot(st['act'][i], w(i, a, b), NT)

        def tick(v):
            st['n'] = st.get('n', 0) + 1
            for r0 in range(PAR1, v.shape[0], 16) if st['n'] % 4 == QPH else ():
                if jobs.tick(lambda: v[r0:r0 + 8], cap=st['cap']):
                    side.now += 1
                else:
                    side.tick(lambda: v[r0:r0 + 8])

        def kdot(a, b, dims=NN):
            if a[0].shape[0] > DH:
                return _cat([kdot([x[DH * q:DH * (q + 1)] for x in a], b, dims) for q in range(2)], 0)
            acc = None
            for x, y in zip(a, b):
                v = _dot(x, y, dims)
                tick(v)
                acc = v if acc is None else acc + v
            return acc

        def proj(k, p):
            Z, ZC = (XN, GT)[k], pb(ZC_, k)
            te, to = _tile(2 * p), _tile(2 * p + 1)
            m = []
            for i in range(7):
                if i == 3:
                    zs = [Z[KM:KM + T, to], _cat([Z[KM + T:KR, to], Z[KR + KQ:KR + 2 * KQ, te]], 0)]
                else:
                    r0, R, c = (KH * SUMI[i], ZC, p) if i in SUMI else (KH * (i - 2), Z, 2 * p + i - 2)
                    zs = [R[r0 + T * q:r0 + T * (q + 1), _tile(c)] for q in range(2)]
                m.append(kdot([WTc[(7 * k + i) * DH:(7 * k + i + 1) * DH, _tile(q)] for q in range(2)], zs))
            c11, c12, c21, c22 = _recombine(m)
            lo, hi, mix = [WTt[DH * u:DH * (u + 1), _tile(k)] for u in range(3)]
            c12 = c12 + kdot([mix], [Z[KR:M, te]])
            c21 = c21 + kdot([lo], [_cat([Z[KR:KR + KQ, to], ZC[KH + KM:2 * KH, _tile(p)], Z[KR + 2 * KQ:M, to]], 0)])
            c22 = c22 + kdot([hi], [Z[KR:M, to]])
            blk = (c11, c12, c21, c22)
            if k == 0:
                blk = [c * (SCALE * LOG2E) for c in blk]
            v = _cat([_cat(blk[0:2], 0), _cat(blk[2:4], 0)])
            QO[_tile(k), 2 * T * p:2 * T * (p + 1)] = v.astype(bf16)
            if p >= 2 and k == 0:
                OUT[k][:, 2 * T * p:2 * T * (p + 1)] = v
            if p % 2 if k == 0 else p > 0:
                HC[5 * DH * k:5 * DH * (k + 1), _tile(p)] = _cat([_comb(i, blk) for i in SUMI], 0).astype(bf16)

        def hk_products(prod, N, left, flip=False):
            quads, singles, pairs = _hk_order(left)
            for r in pairs if flip else ():
                N[:, _tile(r)] = prod(r)
            for quad in quads:
                n = [prod(r) for r in quad]
                for r, v in zip(quad[1:], n[1:]):
                    N[:, _tile(r)] = v
                N[:, _tile(quad[0])] = (n[0] + n[1]) + (n[2] + n[3])
            for r in singles + ([] if flip else pairs):
                N[:, _tile(r)] = prod(r)

        def proj_kv(g):
            WKc, ZD, N = pb(WKc_, z), pb(ZD_, 2), NW.at[z, pl.ds(D * (g % 2), D), :]

            def prod(r):
                i, q = OFFD[r - PN] if r >= PN else (None, None)
                v = _dot(WKc[:, _tile(LSLOT[r])], CT[_tile(i), _tile(NG * g + q)] if r >= PN else ZD[_tile(r), _tile(g)])
                tick(v)
                return v

            if g >= 2:
                jobs.need(('kv', g - 2))
            hk_products(prod, N, False, g % 2)

            def strip(m, r0):
                def put(k0, lo, hi):
                    cols = slice(GW * g + T * k0, GW * g + T * (k0 + 2))
                    for r1, v in ((r0, _cat(lo)), (DH + r0, _cat(hi))):
                        KVT[D * m + r1:D * m + r1 + 16, cols] = v.astype(bf16)
                        if g < NG - 1 and m == 0:
                            OUT[2 + m][r1:r1 + 16, cols] = v
                    if k0 == 0 or (m == 1 and g < NG - 1):
                        for i, sl in SUMI.items():
                            r1 = (5 * (2 + m) + sl) * DH + r0
                            HC[r1:r1 + 16, _tile(2 * g + k0 // 2)] = _comb(i, lo + hi).astype(bf16)
                return _hk_adjoint(lambda a, b: N[DH * m + r0:DH * m + r0 + 16, T * a:T * b], False, put)

            def flip(m, an):
                KV[GW * g:GW * (g + 1), _tile(m)] = gated(KVT[_tile(m), GW * g:GW * (g + 1)], an).T
            jobs.push([fn for m in range(2) for fn in
                       [f for r0 in range(0, DH, 16) for f in strip(m, r0)] + [functools.partial(flip, m)]],
                      KG, KD, ('kv', g))

        src_of = lambda k: (QO, KVT)[k // 2]

        def hop(k, i, p):
            if i in SUMI:
                r0 = (5 * k + SUMI[i]) * DH
                return HC[r0:r0 + DH, _tile(p)]
            r0 = D * (k % 2) + DH * (i - 2)
            return src_of(k)[r0:r0 + DH, _tile(2 * p + i - 2)]

        hh = lambda k, g: pb((Xc_, Yc_)[k // 2], z).at[pl.ds(DH * (3 * (k % 2) + g - (k < 2)), DH), :]

        def side_jobs(k, g):
            def job(r0, kind, s0, s1, an):
                lo, hi = [OUT[k][DH * u + r0:DH * u + r0 + 16, GW * g:GW * (g + 1)] for u in range(2)]
                v = _hk_job(lo, hi, False, kind, an) if k < 2 else _hk_job(hi, lo, True, kind, an)
                hh(k, g)[r0:r0 + 16, T * s0:T * s1] = v.astype(bf16)
            return [functools.partial(job, r0, *hs) for r0 in range(0, DH, 16) for hs in HSETS]

        def sop(k, r, g):
            slot = r if k < 2 else LSLOT[r]
            if slot >= NG:
                return hh(k, g)[:, _tile(slot)]
            r0 = D * (k % 2) + (DH if k < 2 else 0)
            return src_of(k)[r0:r0 + DH, _tile(NG * g + slot)]

        gblk = lambda a, b: _tile(b * (b - 1) // 2 + a)

        def scores():
            c = st['col'] = st.get('col', NC) - 1
            if c < 0:
                return
            assert c + 4 >= NC or ('il', c + 4) in st
            L, Sc = T * (c + 1), Scs[c % 4]
            mx = None
            ss = [_dot(KV[a:b, 0:D], QO[0:D, _tile(c)]) for (a, b) in _chunks(L, L // 4)]
            for k in range(0, L // 64, ATK) if ATK else ():
                jobs.tick(lambda: ss[0][16 * k + PAR1:16 * k + PAR1 + 8], LIGHT, st['cap'])
                side.now += 1
            for s, (a, b) in zip(ss, _chunks(L, L // 4)):
                if b > L - T:
                    d0 = max(a, L - T)
                    r_ = lax.broadcasted_iota(i32, (b - d0, T), 0) + (d0 - (L - T))
                    c_ = lax.broadcasted_iota(i32, (b - d0, T), 1)
                    last = jnp.where(r_ <= c_, s[d0 - a:], -1e9 * LOG2E)
                    s = last if d0 == a else _cat([s[:d0 - a], last], 0)
                Sc[a:b, :] = s
                m = jnp.max(_fold(s), axis=0)
                mx = m if mx is None else jnp.maximum(mx, m)
            m8 = jnp.broadcast_to(jnp.max(mx, axis=0, keepdims=True), (8, T))
            if c >= NC - 4:
                moe_small(4)

            def chunk(a, an):
                p = jnp.exp2(Sc[a:a + BC, :] - _gate(an, [m8], BC))
                P[a:a + BC, _tile(c)] = p.astype(bf16)
                ps = jnp.sum(_fold(p), axis=0)
                st['l', c] = ps if a == 0 else st['l', c] + ps
                if a + BC == L:
                    il = 1.0 / jnp.sum(st['l', c], axis=0, keepdims=True)
                    st['il', c] = il
                    DO2[:, _tile(c)] = (QO[D:2 * D, _tile(c)].astype(f32) * il).astype(bf16)
                    if c % 2 == 0 and c > 0:
                        p_sums(c // 2)
            jobs.push([functools.partial(chunk, a) for a in range(0, L, BC)], delay=DLY)

        def p_sums(b):
            il = [jnp.broadcast_to(st['il', 2 * b + qp], (8, T)) for qp in range(2)]

            def group(a, r0, an):
                sc = _gate(an, il, 16)
                blk = [x for kp in range(2) for x in _tiles(
                    P[T * (2 * a + kp) + r0:T * (2 * a + kp) + r0 + 16, 2 * T * b:2 * T * (b + 1)].astype(f32) * sc)]
                r1 = gblk(a, b).start + r0
                PC[r1:r1 + 16, :] = _cat([_comb(i, blk) for i in range(7)]).astype(bf16)
            jobs.push([functools.partial(group, a, r0) for a in range(b) for r0 in range(0, T, 16)],
                      delay=DLY2, key=('pc', b), front=True)

        def outer(k, g):
            left, src, dst = k < 2, DH4, OUT[(k + 2) % 4]
            gs = range(g + 1, NG) if left else range(g)
            if not gs:
                return
            for o in gs:
                jobs.need(('side', k, o))
            N = NW.at[z, pl.ds(DH * k, DH), :]

            def prod(r):
                v = kdot([sop(k, r, o) for o in gs], [src[gblk(g, o) if left else gblk(o, g), _tile(r)] for o in gs],
                         NT if left else NN)
                return v if r < PR else v * HSC[r]
            hk_products(prod, N, left)
            jobs.need(('side', (k + 2) % 4, g))

            def strip(r0):
                def put(x0, lo, hi):
                    for r1, v in ((r0, lo), (DH + r0, hi)):
                        dst[r1:r1 + 16, GW * g + T * x0:GW * g + T * (x0 + 2)] = _cat(v)
                return _hk_adjoint(lambda a, b: N[r0:r0 + 16, T * a:T * b], left, put)
            jobs.push([f for r0 in range(0, DH, 16) for f in strip(r0)], delay=DLY3, key=('out', k, g), front=True)

        def pair_out(k, b, diag, done):
            left, g = k < 2, b // 2
            if k % 2:
                others = range(b + 1, NP) if left else range(b)
                blk = lambda o, i: PC[gblk(b, o) if left else gblk(o, b), _tile(i)]
            else:
                others = [b ^ 1] if b % 2 != left else []
                blk = lambda o, i: DS[_tile(g), _tile(i)]

            def m(i):
                if left:
                    return kdot([hop(k, BORD[i], o) for o in others], [blk(o, i) for o in others], NT)
                return kdot([hop(k, i, o) for o in others], [blk(o, BORD[i]) for o in others])

            def fin(q, v):
                e, u = (q // 2, q % 2) if left else (q % 2, q // 2)
                d = diag(e, u)
                v = d if v is None else v + d
                if k % 2 == 0 and g != (NG - 1 if left else 0):
                    jobs.need(('out', k, g))
                    v = v + OUT[(k + 2) % 4][DH * u:DH * (u + 1), _tile(2 * b + e)]
                done(e, u, v)
            if not others:
                for q in range(4):
                    fin(q, None)
                return
            m1, m3 = m(1), m(3)
            fin(2, m1 + m3)
            m2, m4 = m(2), m(4)
            c22, c11 = m2 - m1, m3 - m4
            fin(1, m2 + m4)
            m0 = m(0)
            fin(3, c22 + m0 + m(5))
            fin(0, c11 + m0 + m(6))

        def diag_dot(X, r0, W, left, b, e, u):
            es = range(e, 2) if left else range(e + 1)
            return kdot([X[r0 + DH * u:r0 + DH * (u + 1), _tile(2 * b + o)] for o in es],
                        [W(e, o) if left else W(o, e) for o in es], NT if left else NN)

        p_diag = lambda b: lambda kp, qp: P[_tile(2 * b + kp), _tile(2 * b + qp)]
        s_diag = lambda b: lambda kp, qp: DD[_tile(b), _tile(kp + qp)]

        def ctx(b):
            jobs.need(('pc', b) if b else None)

            def done(e, u, v):
                c, rows = 2 * b + e, slice(DH * u, DH * (u + 1))
                O_o[rows, _tile(c)] = v
                part = jnp.sum(_fold(DO2[rows, _tile(c)].astype(f32) * v), axis=0)
                if ('dp', c) in st:
                    st['delta', c] = jnp.sum(st['dp', c] + part, axis=0, keepdims=True)
                st['dp', c] = part
            pair_out(3, b, lambda e, u: diag_dot(KVT, D, p_diag(b), False, b, e, u) * st['il', 2 * b + e], done)

        def store(dst, b, sc):
            def done(e, u, v):
                dst[DH * u:DH * (u + 1), _tile(2 * b + e)] = v if sc is None else v * sc
            return done

        def d_v(a):
            pair_out(1, a, functools.partial(diag_dot, DO2, 0, p_diag(a), True, a), store(dV_o, a, None))

        def d_s(g):
            def ds(rows, c):
                return P[rows, _tile(c)].astype(f32) * (_dot(KV[rows, D:2 * D], DO2[:, _tile(c)]) - st['delta', c])

            def diag(b):
                for i, (kp, qp) in enumerate(((0, 0), (0, 1), (1, 1))):
                    for r0 in (0, DH):
                        r1 = T * (2 * b + kp) + r0
                        DD[T * b + r0:T * b + r0 + DH, _tile(i)] = ds(slice(r1, r1 + DH), 2 * b + qp).astype(bf16)
            pairs = [2 * g, 2 * g + 1]
            if st['n'] % 4 == ALN:
                diag(pairs.pop())
            cols = slice(GW * g, GW * (g + 1))
            delta = _cat([st['delta', NG * g + k] for k in range(NG)])
            for a in range(g):
                v = _cat([KV[GW * a + T * i + r0:GW * a + T * i + r0 + 16, D:2 * D]
                          for r0 in range(0, T, 16) for i in range(NG)], 0)
                dp = _dot(v, DO2[:, cols]).reshape(T // 16, NG, 16, GW)
                c = [_tiles(P[_tile(NG * a + i), cols].astype(f32) * (dp[:, i].reshape(T, GW) - delta))
                     for i in range(NG)]
                DH4[gblk(a, g), :] = _cat([_lin(HW[r], lambda ik: c[ik[0]][ik[1]]) for r in range(NR)]).astype(bf16)
                moe_small(4)
            blk = [ds(_tile(NG * g + kp), NG * g + 2 + qp) for kp in range(2) for qp in range(2)]
            DS[_tile(g), :] = _cat([_comb(i, blk) for i in range(7)]).astype(bf16)
            for b in reversed(pairs):
                diag(b)

        def d_q(b):
            sc = SCALE
            if b == PEND:
                assert len(st['prep']) == 8
                sc = _gate(st['prep'][-1] + st['prep'][-2], [_full(SCALE)], DH)
            pair_out(2, b, functools.partial(diag_dot, KVT, 0, s_diag(b), False, b), store(dQ_o, b, sc))

        def d_k(a):
            pair_out(0, a, functools.partial(diag_dot, QO, 0, s_diag(a), True, a), store(dK_o, a, LN2))

        def push_side(k, g):
            jobs.push(side_jobs(k, g), key=('side', k, g))

        if FAST >= 2:
            moe_small(15)
            moe_small(15)
            dQ_o[0:16, 0:T] = pb(ZC_, t)[_dtile(j, 16), 0:T].astype(f32) + WTc[_dtile(j, 16), 0:T].astype(f32) + pb(WKc_, z)[_dtile(t, 16), 0:T].astype(f32) + WTt[_dtile(t, 16), 0:T].astype(f32)
            return
        todo = {0: list(reversed(range(NP))), 1: list(reversed(range(NP)))}

        def prep():
            def run(job, an):
                done = st.setdefault('prep', [])
                done.append(job(an + done[-2] if len(done) > 1 else an))
            big, small = prep_jobs(jnp.minimum(h + 1, H - 1), z)
            side.push([functools.partial(run, job) for job in big], PGAP)
            side.push(small, 2, 8 * PGAP)

        def step(name, g):
            st['cap'] = CAP['G' if name[0] == 'G' else 'p' if name[0] in 'qo' else 'A' if name == 'A'
                            else ('T' if name[0] in 'KV' else 'H') if name[-1] == 'H' else 'c' if name[0] in 'CV' else 'i']
            if name[0] == 's':
                return push_side(int(name[1]), int(name[2]))
            if name[0] == 'G':
                return proj_kv(int(name[1]))
            if name[0] in 'qo':
                k = 'qo'.index(name[0])
                for _ in range(int(name[1:])):
                    proj(k, todo[k].pop(0))
                return
            if name == 'A':
                jobs.need(('kv', NG - 1))
                return scores()
            if name == 'W':
                return prep()
            if name == 'P':
                return d_s(g)
            if name[1] == 'H':
                return outer('KVEC'.index(name[0]), g)
            return dict(C=ctx, V=d_v, E=d_q, K=d_k)[name[0]](2 * g + int(name[1]))

        for g, names in zip(range(NG, -1, -1), ORD):
            for name in names:
                step(name, g)
        assert not todo[0] and not todo[1] and st['col'] <= 0
        assert not moe1 and not moe2 and not jobs.q and not side.q

    def out_block(j, t):
        z = jnp.minimum(j, 0)
        sl = j & 1
        WC = pb(WC_, z)
        hrs, wrow = (MQ, T), (0, MQ)
        X = ((XF.at[2 * t], XF.at[2 * t + 1]), (YF.at[2 * t], YF.at[2 * t + 1]))
        Xc = (pb(Xc_, z), pb(Yc_, z))
        Zraw, Zsum = (pb(ZR_, t), CT), (pb(ZD_, t), pb(ZD_, 2))
        acc = (AM.at[t], AC)
        keep = (j > 0, jnp.logical_or(j > 0, t == 0))
        N = NW.at[z]
        jobs = _Jobs()

        def tick(v):
            for k in range(8):
                r0 = (k * (v.shape[0] // 16) // 8) * 16 + PAR2
                jobs.tick(lambda: v[r0:r0 + 8, 0:T])

        def x_job(f, kind, s0, s1, g, r0, an):
            u, v = [X[f][hd][r0:r0 + 16, GW * g:GW * (g + 1)] for hd in range(2)]
            Xc[f][D * g + r0:D * g + r0 + 16, T * s0:T * s1] = _hk_job(u, v, False, kind, an).astype(bf16)

        def wa_job(r0, an):
            zero = pltpu.bitcast(_gate(an, [_full(0.0)], 16), u32)
            lo, hi = [pltpu.bitcast(pltpu.bitcast(
                RAW[sl, RO + hd * MH + r0 // 2:RO + hd * MH + r0 // 2 + 16, :] | zero, bf16).astype(f32), u32)
                for hd in range(2)]
            WA[z, r0:r0 + 32, :] = jnp.where(t == 0, RAW[sl, RQ + r0:RQ + r0 + 32, :], (lo >> 16) | hi)

        def w_job(f, kind, s0, s1, r0, an):
            src = WA.at[z] if f == 0 else RAW.at[sl, pl.ds(pl.multiple_of(RK + t * DC, 8), DC), :]
            w = _cat([src[hrs[f] * i + r0:hrs[f] * i + r0 + 16, :] for i in range(NG)])
            WC[wrow[f] + r0:wrow[f] + r0 + 16, T * s0:T * s1] = _hk_job(
                None if kind == 'r' else _half(w, 1), _half(w, 0), True, kind, an).astype(bf16)

        w_jobs = lambda f: [functools.partial(w_job, f, *hs, r0)
                            for r0 in range(0, hrs[f], 16) for hs in (('r', 0, NG),) + HSETS]

        def o_jobs(f, r0):
            rows = slice(wrow[f] + r0, wrow[f] + r0 + 16)
            diag = {}

            def first(an):
                q = _tiles(N[rows, T * PQ:T * PP] * _gate(an, [_full(1.0)] * NG, 16))
                n = _tiles(N[rows, T * PR:T * NR])
                for k in range(NG):
                    diag[k] = q[k]
                    for i in range(NG):
                        if i != k:
                            diag[k] = diag[k] + (n[PAIRS.index((min(i, k), max(i, k)))]
                                                 + n[PN - PR + OFFD.index((i, k))])

            def second(i0, an):
                p = _tiles(N[rows, T * (PP + i0):T * (PP + i0 + 2)])
                n = _tiles(N[rows, T * (PN + 3 * i0):T * (PN + 3 * i0 + 6)])
                one = _gate(an, [_full(1.0)], 16)
                for i in (i0, i0 + 1):
                    tk = n[3 * (i - i0):3 * (i - i0) + 3]
                    tk.insert(i, diag[i] * one)
                    c0 = p[i - i0] + _lin(dict(enumerate(LAM)), lambda k: tk[k])
                    c1 = (tk[0] + tk[1]) + (tk[2] + tk[3])
                    out = slice(hrs[f] * i + r0, hrs[f] * i + r0 + 16)
                    (stA, stB)[f][t, out, :] = _word(c0, c1)
                    if f == 0:
                        stO[t, 0, out, :] = c0.astype(bf16)
                        stO[t, 1, out, :] = c1.astype(bf16)
            return [first, functools.partial(second, 0), functools.partial(second, 2)]

        def moe_jobs(slot, act_slot):
            def job(i, a, an):
                act = ACT[act_slot, TOPC * i:TOPC * (i + 1)]
                act = _cat([_gate(an, [act[0]], 8)[None], act[1:]], 0)
                xb = XB[TOPC * (i // 2):TOPC * (i // 2 + 1), a:a + 16, :]
                v = jnp.sum(xb * _cat([act, act], 1), axis=0)
                wt_out[slot, i, a // 2:a // 2 + 8, :] = pltpu.bitcast(v.astype(bf16), u32)
            return [functools.partial(job, i, a) for i in range(3) for a in range(0, M, 16)]

        xop = lambda f, r: _cat([Xc[f][_tile(g), _tile(r)] for g in range(NG)])

        def dw_unit(f, r):
            hr = hrs[f]
            if r < PN:
                zop = Zsum[f][hr * r:hr * (r + 1), :]
            else:
                i, q = OFFD[r - PN]
                zop = _cat([Zraw[f][hr * i:hr * (i + 1), _tile(NG * g + q)] for g in range(NG)])
            n = _dot(zop, xop(f, r), NT)
            tick(n)
            N[wrow[f]:wrow[f] + hr, _tile(r)] = n if r < PR else n * HSC[r]

        def acc_unit(f, r):
            hr = hrs[f]
            new = _dot(WC[wrow[f]:wrow[f] + hr, _tile(LSLOT[r])], xop(f, r))
            tick(new)
            new = jnp.stack(_tiles(new))
            acc[f][:, hr * r:hr * (r + 1), :] = jnp.where(keep[f], acc[f][:, hr * r:hr * (r + 1), :], 0.0) + new

        if FAST in (1, 3):
            acc[0][0, 0:8, 0:T] = X[0][0][0:8, _dtile(j)] + X[1][0][0:8, _dtile(j)] + ACT[t, j] + Zsum[0][_dtile(j, 16), 0:T].astype(f32)[0:8] + XB[j, 0:8]
            return
        delay = 0
        for f in range(2):
            for hs in HSETS:
                gap = G1 if delay else G0
                jobs.push([functools.partial(x_job, f, *hs, g, r0) for g in range(NG) for r0 in range(0, D, 16)],
                          gap, delay, (f, hs))
                delay += int(gap * NG * D // 16)
        jobs.push([functools.partial(wa_job, r0) for r0 in range(0, M, 32)], 5, 60)
        jobs.push(w_jobs(0), G2, WD, 'wa')
        jobs.push(w_jobs(1), G6, WD1, 'wb')
        jobs.sort()
        for f in range(2):
            for i in range(NG):
                for g in range(NG):
                    Xc[f][_tile(g), _tile(i)] = X[f][1][:, _tile(NG * g + i)].astype(bf16)
                dw_unit(f, i)
        for f in range(2):
            for hs in HSETS:
                jobs.need((f, hs))
                for r in range(hs[1], hs[2]):
                    dw_unit(f, r)
            jobs.push([fn for r0 in range(0, hrs[f], 16) for fn in o_jobs(f, r0)], (G4, G5)[f], (OD0, OD1)[f])
            jobs.sort()
        kx = jnp.clip(2 * (j - 1) + t, 0, NX - 1)
        jobs.push(moe_jobs(t, t) + moe_jobs(2 + t, jnp.where(j == H // 2 - 1, 1 - t, 2 + kx)), G3, 1)
        jobs.sort()
        for f in range(2):
            jobs.need(('wa', 'wb')[f])
            for r in range(NR):
                acc_unit(f, r)
        assert not jobs.q

        @pl.when(jnp.logical_and(t == 0, j + 2 < H // 2))
        def _():
            w_start(j + 2)

    o_copy = lambda g: copy(XS.at[:, grp(g)], outT_hbm.at[:, grp(g)], sem_out.at[0])
    dx_copy = lambda g: copy(DX.at[:, grp(g)], dxT_hbm.at[:, grp(g)], sem_out.at[1])
    dc_copy = lambda g: copy(CS.at[grp(g), :], dc_hbm.at[grp(g), :], sem_out.at[2])

    def acc_rows(acc, hr, i, r0, n):
        ld = functools.lru_cache(None)(lambda r: acc[hr * r + r0:hr * r + r0 + n, :])
        return _cat([_lin({r: HW[r][i, q] * HSC[r] for r in range(NR) if (i, q) in HW[r]}, ld) for q in range(NG)])

    def finish_out():
        for cp in grad_copies(H // 2 - 1, 1):
            cp.start()
        to_start(1, H - 1)
        to_start(3, H - 2)
        updT[...] = (_rb(yacc[...]) * srt[:, 0:1]).T.astype(bf16)

        def o_step(g, carry):
            oh = onehot[:, grp(g)].astype(bf16)
            acc, xs, xn = AM.at[1, g], XS.at[:, grp(g)], XN.at[:, grp(g)]
            for i in range(NG):
                so = _dot(updT[MQ * i:MQ * (i + 1), :], oh)
                for r0 in range(0, MQ, 16):
                    rows = slice(MQ * i + r0, MQ * i + r0 + 16)
                    xs[rows, :] = (xs[rows, :].astype(f32) + xn[rows, :].astype(f32)
                                   + acc_rows(acc, MQ, i, r0, 16) + so[r0:r0 + 16]).astype(bf16)
            o_copy(g).start()
            return carry
        lax.fori_loop(0, NG, o_step, None)

    def pair_step(j, carry):
        @pl.when(j == 1)
        def _():
            for cp in fi_copies():
                cp.wait()
            moe_chunk()

        def hb(t, c):
            head_block(j, t)
            return c
        lax.fori_loop(0, 2, hb, None)

        @pl.when(j > 0)
        def _():
            to_wait(0)
            to_wait(1)
            for cp in grad_copies(j - 1, 0) + grad_copies(j - 1, 1):
                cp.wait()

        @pl.when(jnp.logical_and(j >= 2, j < 2 + NX // 2))
        def _():
            to_wait(2)
            to_wait(3)

        def ob(t, c):
            out_block(j, 1 - t)

            @pl.when(jnp.logical_and(j == H // 2 - 1, t == 0))
            def _():
                finish_out()
            return c
        lax.fori_loop(0, 2, ob, None)
        return carry
    lax.fori_loop(0, H // 2, pair_step, None)

    for cp in grad_copies(H // 2 - 1, 0):
        cp.start()

    def dc_part(g):
        acc, out = AC.at[g], CS.at[grp(g), :]
        for i in range(NG):
            out[:, _tile(i)] = _cat([acc_rows(acc, T, i, r0, 32) for r0 in range(0, T, 32)], 0).astype(bf16).T

    dc_part(0)
    s_r = srt[:, 0:1]
    dr = _rb(_rb(jnp.sum(selacc[1] * _rb(yacc[...]), axis=1, keepdims=True)) * _rb(s_r * _rb(1.0 - s_r)))
    dwr_ref[...] = jnp.sum(dr * selacc[0], axis=0).astype(bf16)
    dxsT[...] = (dxacc[...] + dr * wr_ref[...].astype(f32).reshape(1, M)).T.astype(bf16)
    dc_copy(0).start()
    dwr_copy = copy(dwr_ref, dwr_hbm, sem_out.at[3])
    dwr_copy.start()

    def dx_step(g, last):
        tmp = TMP.at[jnp.minimum(g, 0)]
        oh = onehot[:, grp(g)].astype(bf16)
        acc, gt, xn, dxo = AM.at[0, g], GT.at[:, grp(g)], XN.at[:, grp(g)], DX.at[:, grp(g)]
        rs = rstd[0:1, grp(g)]
        s1 = s2 = 0.0
        for i in range(NG):
            sx = _dot(dxsT[MQ * i:MQ * (i + 1), :], oh)
            for r0 in range(0, MQ, 16):
                rows = slice(MQ * i + r0, MQ * i + r0 + 16)
                gr = gt[rows, :].astype(f32)
                dxn = gr + acc_rows(acc, MQ, i, r0, 16) + sx[r0:r0 + 16]
                tmp[rows, :] = dxn * rs + gr
                s1 = s1 + jnp.sum(_fold(dxn), axis=0)
                s2 = s2 + jnp.sum(_fold(dxn * xn[rows, :].astype(f32)), axis=0)
        m1 = jnp.sum(s1, axis=0, keepdims=True) * (rs * (1.0 / M))
        m2 = jnp.sum(s2, axis=0, keepdims=True) * (rs * (1.0 / M))
        tmp2, xn2 = TMP.at[jnp.minimum(2 * g, 0)], pb(ZR_, jnp.minimum(g, 0)).at[:, grp(g)]
        for r0 in range(0, M, 16):
            rows = slice(r0, r0 + 16)
            dxo[rows, :] = (tmp2[rows, :] - m1 - xn2[rows, :].astype(f32) * m2).astype(bf16)

    def fin_step(g, carry):
        dx_step(g, False)
        dx_copy(g).start()

        @pl.when(g + 1 < NG)
        def _():
            dc_part(g + 1)
            dc_copy(g + 1).start()
        return carry
    lax.fori_loop(0, NG, fin_step, None)
    to_wait(1)
    to_wait(3)
    for cp in grad_copies(H // 2 - 1, 0) + grad_copies(H // 2 - 1, 1):
        cp.wait()
    dwr_copy.wait()
    copy(XS, outT_hbm, sem_out.at[0]).wait()
    copy(CS, dc_hbm, sem_out.at[2]).wait()
    copy(DX, dxT_hbm, sem_out.at[1]).wait()


@jax.jit
def pallas_parallel_sum__compressed_kv_cla__moe_arch_mod__prompt_kernel(
        A_x, A_c_kv, A_w_q, A_w_uk, A_w_uv, A_w_o, B_x, B_w_r, B_w_gate, B_w_up, B_w_down, grad_out):
    del B_x
    xT = A_x.reshape(S, M).T
    gT = grad_out.reshape(S, M).T
    c = A_c_kv.reshape(S, DC)
    woT = jnp.swapaxes(A_w_o, 1, 2)
    wdT = B_w_down.T

    ANY = pl.BlockSpec(memory_space=pl.ANY)
    V = pltpu.VMEM
    pb = lambda n, r, c_: V((n, r // 2, c_), u32)
    sds = jax.ShapeDtypeStruct
    dma = pltpu.SemaphoreType.DMA
    outs = pl.pallas_call(
        _kernel,
        in_specs=[ANY] * 11,
        out_specs=[ANY] * 11,
        out_shape=[sds((M, S), bf16), sds((M, S), bf16), sds((S, DC), bf16),
                   sds((M, H, D), bf16), sds((DC, H, D), bf16), sds((DC, H, D), bf16),
                   sds((H, M, D), bf16), sds((M,), bf16),
                   sds((M, F), bf16), sds((M, F), bf16), sds((M, F), bf16)],
        scratch_shapes=[
            pb(1, M, S), pb(1, M, S), pb(1, S, DC),
            pb(2, M, S), pb(1, DC, S), pb(2, 5 * KH, HS), pb(3, PN * MQ, GW),
            V((8, S), f32), V((2, NG, NR * MQ, T), f32), V((NG, NR * T, T), f32),
            V((1, M, GW), f32), V((1, MQ + T, NR * T), f32),
            V((2, 2 * M + 2 * DC, D), u32), V((1, M, D), u32),
            pb(1, 14 * DH, KH), pb(1, 3 * DH, 2 * T), V((1, 2 * D, DC), f32), pb(1, D, NR * T),
            pb(1, 2 * MQ, NR * T),
            pb(1, S, 2 * D), pb(1, 2 * D, S), pb(1, 2 * D, S), pb(1, D, S),
            V((1, S, T), f32), V((1, S, T), f32), V((1, S, T), f32), V((1, S, T), f32),
            pb(1, S, S), pb(1, NBLK * T, NR * T),
            pb(1, NP * (NP - 1) // 2 * T, 7 * T), pb(1, NG * T, 7 * T),
            pb(1, NP * T, 3 * T), pb(1, 20 * DH, HS),
            V((4, D, S), f32), V((4, D, S), f32),
            pb(1, NG * D, NR * T), pb(1, NG * D, NR * T),
            V((2, M, D), u32), V((2, DC, D), u32), V((2, 2, M, D), bf16),
            pb(3, M, FC), V((2, 3, MH, T), u32), V((4, 3, MH, T), u32),
            V((2 * TOPC, M, T), f32), V((2 + NX, 3 * TOPC, 8, T), f32),
            V((8, S), f32), V((8, S), f32), V((CP, S), f32), V((2, CP, M), f32),
            V((CP, M), bf16), V((CP, M), bf16), V((M, CP), bf16), V((M, CP), bf16),
            V((CP, T), f32), V((CP, M), f32), V((CP, M), f32),
            V((M,), bf16), V((M,), bf16), pltpu.SMEM((TOPC,), i32),
            dma((NP,)), dma((2,)), dma((4,)), dma((1,)), dma((2,)), dma((4,)), dma((4,)),
        ],
        compiler_params=pltpu.CompilerParams(vmem_limit_bytes=120 * 1024 * 1024, disable_bounds_checks=bool(int(_env("NOBC", 1)))),
    )(xT, gT, c, A_w_q, A_w_uk, A_w_uv, woT, B_w_r, B_w_gate, B_w_up, wdT)
    outT, dxT, dc, dwq, dwuk, dwuv, dwoT, dwr, dwg, dwu, dwdT = outs
    return (outT.T[None], dxT.T[None], dc[None], dwq, dwuk, dwuv, jnp.swapaxes(dwoT, 1, 2), dwr, dwg, dwu, dwdT.T)
```
